```python
import os as _os
_os.environ.setdefault("JAX_PLATFORMS", "cpu")
import jax
import jax.numpy as jnp

def _softmax(x, axis=-1):
    return jax.nn.softmax(x, axis=axis)
def _gelu(x):
    return jax.nn.gelu(x, approximate=True)
def _silu(x):
    return jax.nn.silu(x)
def _sigmoid(x):
    return jax.nn.sigmoid(x)
def _layernorm(x, axis=-1, eps=1e-5):
    m = jnp.mean(x, axis=axis, keepdims=True)
    v = jnp.var(x, axis=axis, keepdims=True)
    return (x - m) / jnp.sqrt(v + eps)
def _scatter_add(tgt, idx, src, axis=0):
    return tgt.at[idx].add(src)
def _segment_sum(src, seg, n):
    return jax.ops.segment_sum(src, seg, n)
class _Rng:
    def __init__(self, key):
        self._k = key
    def _next(self):
        self._k, sub = jax.random.split(self._k)
        return sub
    def normal(self, shape):
        return jax.random.normal(self._next(), shape, dtype=jnp.bfloat16)
    def randint(self, lo, hi, shape):
        return jax.random.randint(self._next(), shape, lo, hi, dtype=jnp.int32)
    def uniform(self, shape, lo=0.0, hi=1.0):
        return jax.random.uniform(self._next(), shape, jnp.bfloat16, lo, hi)
    def permutation(self, n):
        return jax.random.permutation(self._next(), n)


kernel_name = 'parallel_sum__ssm_conv_s5__glu_gated_swiglu__prompt'

def setup_inputs():
    _rng = _Rng(jax.random.key(int.from_bytes(__import__("os").urandom(4), "little")))
    _w = (lambda a: (lambda t: t.astype(jnp.bfloat16) if jnp.issubdtype(t.dtype, jnp.floating) else t)(jnp.asarray(a)))
    def _A_setup():
        B, S, D = 1, 2048, 640
        P = D
        Lambda_re = -0.5 * jnp.exp((lambda *s: _rng.normal(s) * 0.4)(P))
        Lambda_im = (lambda *s: _rng.normal(s) * 0.4)(P) * 1.0
        B_re = (lambda *s: _rng.normal(s) * 0.4)(P, D) * (D ** -0.5)
        B_im = (lambda *s: _rng.normal(s) * 0.4)(P, D) * (D ** -0.5)
        C_re = (lambda *s: _rng.normal(s) * 0.4)(D, P) * (P ** -0.5)
        C_im = (lambda *s: _rng.normal(s) * 0.4)(D, P) * (P ** -0.5)
        log_dt = (lambda *s: _rng.normal(s) * 0.4)(P) * 0.3 - 2.0
        Dskip = (lambda *s: _rng.normal(s) * 0.4)(D)
        return {
            "x": _w((lambda *s: _rng.normal(s) * 0.05)(B, S, D)),
            "Lambda_re": _w(Lambda_re),
            "Lambda_im": _w(Lambda_im),
            "B_re": _w(B_re),
            "B_im": _w(B_im),
            "C_re": _w(C_re),
            "C_im": _w(C_im),
            "log_dt": _w(log_dt),
            "Dskip": _w(Dskip),
        }
    _A_in = _A_setup()

    def _B_setup():
        B, S, D, F = 1, 2048, 640, 1728
        return {
            "x": _w((lambda *s: _rng.normal(s) * 0.05)(B, S, D)),
            "w1": _w((lambda *s: _rng.normal(s) * 0.1)(D, F) * (2.0 / D) ** 0.5),
            "w3": _w((lambda *s: _rng.normal(s) * 0.1)(D, F) * (2.0 / D) ** 0.5),
            "w2": _w((lambda *s: _rng.normal(s) * 0.1)(F, D) * (2.0 / F) ** 0.5),
        }
    _B_in = _B_setup()

    return {
        "A_x": _A_in["x"],
        "A_Lambda_re": _A_in["Lambda_re"],
        "A_Lambda_im": _A_in["Lambda_im"],
        "A_B_re": _A_in["B_re"],
        "A_B_im": _A_in["B_im"],
        "A_C_re": _A_in["C_re"],
        "A_C_im": _A_in["C_im"],
        "A_log_dt": _A_in["log_dt"],
        "A_Dskip": _A_in["Dskip"],
        "B_x": _B_in["x"],
        "B_w1": _B_in["w1"],
        "B_w3": _B_in["w3"],
        "B_w2": _B_in["w2"],
    }

def reference(A_x, A_Lambda_re, A_Lambda_im, A_B_re, A_B_im, A_C_re, A_C_im, A_log_dt, A_Dskip, B_x, B_w1, B_w3, B_w2):
    def _A_ref(x, Lambda_re, Lambda_im, B_re, B_im, C_re, C_im, log_dt, Dskip):
        Bsz, L, H = x.shape
        Lam = Lambda_re + 1j * Lambda_im
        Bmat = B_re + 1j * B_im
        Cmat = C_re + 1j * C_im
        dt = jnp.exp(log_dt)
        Lam_bar = jnp.exp(dt * Lam)
        B_bar = ((Lam_bar - 1.0) / Lam)[:, None] * Bmat
        Bu = jnp.einsum("bld,pd->blp", x + 0j, B_bar)
        h = jnp.zeros_like(Bu[:, 0, :])
        hs = []
        for t in range(L):
            h = Lam_bar[None, :] * h + Bu[:, t, :]
            hs.append(h)
        hseq = jnp.stack(hs, 1)
        y = 2.0 * jnp.einsum("blp,dp->bld", hseq, Cmat).real + x * Dskip[None, None, :]
        return y

    def _B_ref(x, w1, w3, w2):
        gate = jnp.einsum("bsd,df->bsf", x, w1)
        up = jnp.einsum("bsd,df->bsf", x, w3)
        h = _silu(gate) * up
        out = jnp.einsum("bsf,fd->bsd", h, w2)
        return out

    x = A_x
    xn = _layernorm(x, axis=-1)
    return x + _A_ref(xn, A_Lambda_re, A_Lambda_im, A_B_re, A_B_im, A_C_re, A_C_im, A_log_dt, A_Dskip) + _B_ref(xn, B_w1, B_w3, B_w2)
```

```python
import functools

import jax
import jax.numpy as jnp
from jax import lax
import jax.experimental.pallas as pl
import jax.experimental.pallas.tpu as pltpu

T0 = 416
T = 272
NT_DIMS = (((1,), (1,)), ((), ()))
F32 = jnp.float32
BF16 = jnp.bfloat16
I32 = jnp.int32


def _bf(v):
    return v.astype(BF16).astype(F32)


def _dot_nt(a, b):
    return lax.dot_general(a, b, NT_DIMS, preferred_element_type=F32)


def _dot(a, b):
    return jnp.dot(a, b, preferred_element_type=F32)


def _silu_mul(g, u):
    return (g * jax.nn.sigmoid(g) * u).astype(BF16)


def _cpow(pr, pi, n):
    rr, ri = None, None
    while n:
        if n & 1:
            if rr is None:
                rr, ri = pr, pi
            else:
                rr, ri = rr * pr - ri * pi, rr * pi + ri * pr
        n >>= 1
        if n:
            pr, pi = pr * pr - pi * pi, 2.0 * pr * pi
    return rr, ri


def _cdiv(ar, ai, br, bi):
    swap = jnp.abs(br) < jnp.abs(bi)
    p = jnp.where(swap, bi, br)
    q = jnp.where(swap, br, bi)
    r = q / p
    den = p + q * r
    x = jnp.where(swap, ai, ar)
    y = jnp.where(swap, ar, ai)
    re = (x + y * r) / den
    im = (y - x * r) / den
    return re, jnp.where(swap, -im, im)


def _or_all(v):
    b = pltpu.bitcast(v, I32)
    n, d = b.shape
    parts = [b[r:r + 8, c:c + 128] for r in range(0, n, 8) for c in range(0, d, 128)]
    while len(parts) > 1:
        parts = [parts[i] | parts[i + 1] if i + 1 < len(parts) else parts[i]
                 for i in range(0, len(parts), 2)]
    return parts[0]


def _zero(b):
    return jnp.minimum(lax.shift_right_logical(b, 1), 0).astype(F32)


def _add_top(v, z):
    return jnp.concatenate([v[0:8, :] + z, v[8:, :]], axis=0)


def _kernel(x_hbm, lre_hbm, lim_hbm, ldt_hbm, dsk_hbm, bre_hbm, bim_hbm, cre_hbm, cim_hbm,
            w1t_hbm, w3t_hbm, w2_hbm, o_hbm,
            xv, lre_v, lim_v, ldt_v, dsk_v, wa, craw, cp, w2s,
            xs, xn_ref, base_cur, base_nxt, hh_ref, u_ref, g_ref, par_ref, dskf, carry_ref, ost,
            sem, osem, *, L, D, P, F):
    NC = D // 128
    NLOOP = (L - T0) // T
    assert T0 + NLOOP * T == L
    FM = (F // 128) * 128
    FR = F - FM
    assert FM == 13 * 128 and 2 * FR == 128 and P == 5 * 128

    cnt = [0]

    def cp_(src, dst):
        c = pltpu.make_async_copy(src, dst, sem.at[cnt[0]])
        cnt[0] += 1
        return c

    rows = lambda ref, s, n: ref.at[pl.ds(s, n)]

    pos = [0]
    where = {}

    def wpiece(name, src, a, b):
        n = b - a
        c = cp_(rows(src, a, n), rows(wa, pos[0], n))
        where[name] = (pos[0], pos[0] + n)
        pos[0] += n
        return c

    c128 = lambda a: a * 128
    gv = [cp_(s, d) for s, d in [(dsk_hbm, dsk_v), (lre_hbm, lre_v), (lim_hbm, lim_v), (ldt_hbm, ldt_v)]]
    g0 = [cp_(rows(x_hbm, 0, T0), rows(xv, 0, T0))]
    g1 = [wpiece("g0", w1t_hbm, 0, c128(4))]
    e1 = pos[0]
    g2 = [wpiece("u0", w3t_hbm, 0, c128(4)), wpiece("g1", w1t_hbm, c128(4), c128(8))]
    e2 = pos[0]
    g3 = [wpiece("u1", w3t_hbm, c128(4), c128(8)), wpiece("g2", w1t_hbm, c128(8), c128(11)),
          wpiece("bre", bre_hbm, 0, P)]
    e3 = pos[0]
    g4 = [wpiece("bim", bim_hbm, 0, P), wpiece("u2", w3t_hbm, c128(8), c128(11)),
          wpiece("g3", w1t_hbm, c128(11), FM), wpiece("u3", w3t_hbm, c128(11), FM)]
    e4 = pos[0]
    g4 += [wpiece("gr", w1t_hbm, FM, F), wpiece("ur", w3t_hbm, FM, F)]
    e5 = pos[0]
    g5 = [cp_(w2_hbm, w2s), cp_(cre_hbm, craw.at[0]), cp_(cim_hbm, craw.at[1])]
    XS0 = cnt[0]
    B0 = where["bre"][0]
    B1 = where["bim"][1]

    def x_copy(k):
        s = T0 + k * T
        if not isinstance(k, int):
            s = pl.multiple_of(s, 16)
        return pltpu.make_async_copy(rows(x_hbm, s, T), rows(xv, s, T), sem.at[XS0 + k])

    def out_copy(start, n, c, k):
        return pltpu.make_async_copy(
            ost.at[c, pl.ds(start, n)], o_hbm.at[pl.ds(start, n), pl.ds(c * 128, 128)], osem.at[k])

    def ln_stage_in(start, n):
        xf = xv[pl.ds(start, n), :].astype(F32)
        for c in range(NC):
            xs[c, 0:n, :] = xf[:, c * 128:(c + 1) * 128]

    def ln_pieces(n, base_ref, q0, q1, ntok=0):
        seg = n // 8
        toks = [None] * ntok
        for q in range(q0, q1):
            j = 2 * q
            xp = jnp.concatenate(
                [jnp.concatenate([xs[c, pl.ds(jj, 8, stride=seg), :] for jj in (j, j + 1)], axis=0)
                 for c in range(NC)], axis=1)
            mean = jnp.mean(xp, axis=-1, keepdims=True)
            xc32 = xp - mean
            var = jnp.mean(xc32 * xc32, axis=-1, keepdims=True)
            den = _bf(jnp.sqrt(_bf(_bf(var) + 1e-5)))
            xnb = (_bf(xp - _bf(mean)) * (1.0 / den)).astype(BF16)
            xn_ref[j * 8:(j + 2) * 8, :] = xnb
            base = xp + xnb.astype(F32) * dskf[0:1, :]
            base_ref[j * 8:(j + 2) * 8, :] = base
            if ntok:
                p = (q - q0) * ntok // (q1 - q0)
                b = _or_all(base)
                toks[p] = b if toks[p] is None else toks[p] | b
        if ntok:
            toks = [_zero(t) for t in toks]
            return (jnp.concatenate(toks[0:NC], axis=1), jnp.concatenate(toks[NC:2 * NC], axis=1))

    def ln_next(start):
        ln_stage_in(start, T)
        return ln_pieces(T, base_nxt, 0, T // 16, 2 * NC)

    def param_stage():
        lre = lre_v[...].astype(F32).reshape(1, P)
        lim = lim_v[...].astype(F32).reshape(1, P)
        dt = _bf(jnp.exp(ldt_v[...].astype(F32).reshape(1, P)))
        er = jnp.exp(dt * lre)
        are = er * jnp.cos(dt * lim)
        aim = er * jnp.sin(dt * lim)
        kre, kim = _cdiv(are - 1.0, aim, lre, lim)
        par_ref[0] = jnp.broadcast_to(are, (8, P))
        par_ref[1] = jnp.broadcast_to(aim, (8, P))
        for t, off in ((T0, 2), (T, 8)):
            pr, pi = _cpow(are, aim, t // 8)
            for k in range(3):
                par_ref[off + 2 * k] = jnp.broadcast_to(pr, (8, P))
                par_ref[off + 1 + 2 * k] = jnp.broadcast_to(pi, (8, P))
                pr, pi = pr * pr - pi * pi, 2.0 * pr * pi
        par_ref[14] = jnp.broadcast_to(2.0 * kre, (8, P))
        par_ref[15] = jnp.broadcast_to(2.0 * kim, (8, P))
        carry_ref[...] = jnp.zeros_like(carry_ref)

    def cprep_stage():
        kre = par_ref[14, 0:1, :]
        kim = par_ref[15, 0:1, :]
        cre = craw[0].astype(F32)
        cim = craw[1].astype(F32)
        cp[:, 0:P] = (cre * kre - cim * kim).astype(BF16)
        cp[:, P:2 * P] = (-(cre * kim) - cim * kre).astype(BF16)

    def scan_stage(n, off):
        seg = n // 8
        are = par_ref[0]
        aim = par_ref[1]
        er = u_ref[0:8, 0:P]
        ei = u_ref[0:8, P:2 * P]
        for j in range(1, seg):
            ur = u_ref[j * 8:(j + 1) * 8, 0:P]
            ui = u_ref[j * 8:(j + 1) * 8, P:2 * P]
            er, ei = (are * er - aim * ei) + ur, (are * ei + aim * er) + ui
        row = lax.broadcasted_iota(I32, (8, P), 0)
        zr = jnp.where(row == 0, pltpu.roll(carry_ref[0], 1, 0), pltpu.roll(er, 1, 0))
        zi = jnp.where(row == 0, pltpu.roll(carry_ref[1], 1, 0), pltpu.roll(ei, 1, 0))
        for k in range(3):
            d = 1 << k
            pr = par_ref[off + 2 * k]
            pi = par_ref[off + 1 + 2 * k]
            sr = jnp.where(row >= d, pltpu.roll(zr, d, 0), 0.0)
            si = jnp.where(row >= d, pltpu.roll(zi, d, 0), 0.0)
            zr, zi = zr + (pr * sr - pi * si), zi + (pr * si + pi * sr)
        hr, hi = zr, zi
        for j in range(0, seg, 2):
            outs_r = []
            outs_i = []
            for jj in (j, j + 1):
                ur = u_ref[jj * 8:(jj + 1) * 8, 0:P]
                ui = u_ref[jj * 8:(jj + 1) * 8, P:2 * P]
                hr, hi = (are * hr - aim * hi) + ur, (are * hi + aim * hr) + ui
                outs_r.append(hr)
                outs_i.append(hi)
            g_ref[j * 8:(j + 2) * 8, 0:P] = jnp.concatenate(outs_r, axis=0).astype(BF16)
            g_ref[j * 8:(j + 2) * 8, P:2 * P] = jnp.concatenate(outs_i, axis=0).astype(BF16)
        carry_ref[0] = hr
        carry_ref[1] = hi

    def out_stage(start, n, k, res):
        seg = n // 8
        for c in range(NC):
            for j in range(seg):
                ost[c, pl.ds(start + j, 8, stride=seg), :] = res[j * 8:(j + 1) * 8, c * 128:(c + 1) * 128]
            out_copy(start, n, c, k).start()

    def sl(r, base, name):
        a, b = where[name]
        return r[:, a - base:b - base]

    for grp in (gv, g0, g1, g2, g3, g4, g5):
        for c in grp:
            c.start()
    for k in range(NLOOP):
        x_copy(k).start()

    def wait(grp):
        for c in grp:
            c.wait()

    xdot = lambda a, b, r0=0, r1=T0: _dot_nt(xn_ref[r0:r1, :], wa[a:b, :])

    wait(gv)
    dskf[...] = jnp.broadcast_to(dsk_v[...].astype(F32).reshape(1, D), (8, D))
    param_stage()
    wait(g0)
    ln_stage_in(0, T0)
    NP0 = T0 // 16
    H = NP0 // 2
    ln_pieces(T0, base_cur, 0, H)
    wait(g1)
    ra = xdot(0, e1, 0, H * 16)
    ln_pieces(T0, base_cur, H, NP0)
    rb = xdot(0, e1, H * 16, T0)
    r1 = jnp.concatenate([ra, rb], axis=0)
    wait(g2)
    r2 = xdot(e1, e2)
    hh_ref[:, c128(0):c128(4)] = _silu_mul(r1, sl(r2, e1, "u0"))
    wait(g3)
    r3 = xdot(e2, e3)
    hh_ref[:, c128(4):c128(8)] = _silu_mul(sl(r2, e1, "g1"), sl(r3, e2, "u1"))
    u_ref[0:T0, 0:P] = sl(r3, e2, "bre")
    wait(g4)
    r4 = xdot(e3, e4)
    u_ref[0:T0, P:2 * P] = sl(r4, e3, "bim")
    scan_stage(T0, 2)
    qs = [0] + [((T0 * i // 4) + 15) // 16 * 16 for i in (1, 2, 3)] + [T0]
    rr = jnp.concatenate([xdot(e4, e5, qs[i], qs[i + 1]) for i in range(4)], axis=0)
    hh_ref[:, FM:F] = _silu_mul(rr[:, 0:FR], rr[:, FR:2 * FR])
    hh_ref[:, c128(8):c128(11)] = _silu_mul(sl(r3, e2, "g2"), sl(r4, e3, "u2"))
    hh_ref[:, c128(11):FM] = _silu_mul(sl(r4, e3, "g3"), sl(r4, e3, "u3"))
    wait(g5)
    x_copy(0).wait()
    cprep_stage()
    z1, z2 = ln_next(T0)
    acc = _add_top(base_cur[0:T0, :] + _dot(hh_ref[...], w2s[...]), z1)
    acc = _add_top(acc + _dot_nt(g_ref[0:T0, :], cp[...]), z2)
    out_stage(0, T0, 0, acc)

    def body(k, carry):
        kn = jnp.minimum(k + 1, NLOOP - 1)

        @pl.when(k + 1 < NLOOP)
        def _():
            x_copy(kn).wait()

        start = pl.multiple_of(T0 + k * T, 16)
        nxt = pl.multiple_of(T0 + kn * T, 16)
        xnb = xn_ref[0:T, :]
        u_ref[0:T, :] = _dot_nt(xnb, wa[B0:B1, :])
        base_cur[0:T, :] = base_nxt[...]
        scan_stage(T, 8)
        ra = _dot_nt(xnb, wa[0:B0, :])
        rb = _dot_nt(xnb, wa[B1:e5, :])
        hh = jnp.concatenate([
            _silu_mul(sl(ra, 0, "g0"), sl(ra, 0, "u0")),
            _silu_mul(sl(ra, 0, "g1"), sl(ra, 0, "u1")),
            _silu_mul(sl(ra, 0, "g2"), sl(rb, B1, "u2")),
            _silu_mul(sl(rb, B1, "g3"), sl(rb, B1, "u3")),
            _silu_mul(sl(rb, B1, "gr"), sl(rb, B1, "ur")),
        ], axis=1)
        z1, z2 = ln_next(nxt)
        acc = _add_top(base_cur[0:T, :] + _dot(hh, w2s[...]), z1)
        acc = _add_top(acc + _dot_nt(g_ref[0:T, :], cp[...]), z2)
        out_stage(start, T, k + 1, acc)
        return carry

    lax.fori_loop(0, NLOOP, body, 0)

    for c in range(NC):
        out_copy(0, T0, c, 0).wait()
    for k in range(NLOOP):
        for c in range(NC):
            out_copy(T0 + k * T, T, c, k + 1).wait()


@jax.jit
def pallas_parallel_sum__ssm_conv_s5__glu_gated_swiglu__prompt_kernel(
    A_x, A_Lambda_re, A_Lambda_im, A_B_re, A_B_im, A_C_re, A_C_im, A_log_dt, A_Dskip,
    B_x, B_w1, B_w3, B_w2,
):
    Bsz, L, D = A_x.shape
    P = A_Lambda_re.shape[0]
    F = B_w1.shape[1]
    NLOOP = (L - T0) // T
    TM = max(T0, T)
    hbm = pl.BlockSpec(memory_space=pltpu.HBM)
    out = pl.pallas_call(
        functools.partial(_kernel, L=L, D=D, P=P, F=F),
        in_specs=[hbm] * 12,
        out_specs=hbm,
        out_shape=jax.ShapeDtypeStruct((L, D), F32),
        scratch_shapes=[
            pltpu.VMEM((L, D), BF16),
            pltpu.VMEM((P,), BF16), pltpu.VMEM((P,), BF16), pltpu.VMEM((P,), BF16), pltpu.VMEM((D,), BF16),
            pltpu.VMEM((2 * P + 2 * F, D), BF16),
            pltpu.VMEM((2, D, P), BF16),
            pltpu.VMEM((D, 2 * P), BF16),
            pltpu.VMEM((F, D), BF16),
            pltpu.VMEM((D // 128, TM, 128), F32),
            pltpu.VMEM((TM, D), BF16),
            pltpu.VMEM((TM, D), F32),
            pltpu.VMEM((T, D), F32),
            pltpu.VMEM((T0, F), BF16),
            pltpu.VMEM((TM, 2 * P), F32),
            pltpu.VMEM((TM, 2 * P), BF16),
            pltpu.VMEM((16, 8, P), F32),
            pltpu.VMEM((8, D), F32),
            pltpu.VMEM((2, 8, P), F32),
            pltpu.VMEM((D // 128, L, 128), F32),
            pltpu.SemaphoreType.DMA((20 + NLOOP,)),
            pltpu.SemaphoreType.DMA((NLOOP + 1,)),
        ],
        compiler_params=pltpu.CompilerParams(
            vmem_limit_bytes=100 * 1024 * 1024,
            disable_bounds_checks=True,
            disable_semaphore_checks=True,
        ),
    )(A_x.reshape(L, D), A_Lambda_re, A_Lambda_im, A_log_dt, A_Dskip,
      A_B_re, A_B_im, A_C_re, A_C_im, B_w1.T, B_w3.T, B_w2)
    return out.reshape(Bsz, L, D)
```

```python
import functools

import jax
import jax.numpy as jnp
from jax import lax
import jax.experimental.pallas as pl
import jax.experimental.pallas.tpu as pltpu

T0 = 416
T = 272
PARK = 4
NT_DIMS = (((1,), (1,)), ((), ()))
F32 = jnp.float32
BF16 = jnp.bfloat16
I32 = jnp.int32


def _bf(v):
    return v.astype(BF16).astype(F32)


def _dot_nt(a, b):
    return lax.dot_general(a, b, NT_DIMS, preferred_element_type=F32)


def _dot(a, b):
    return jnp.dot(a, b, preferred_element_type=F32)


def _silu_mul(g, u):
    return (g * jax.nn.sigmoid(g) * u).astype(BF16)


def _cpow(pr, pi, n):
    rr, ri = None, None
    while n:
        if n & 1:
            if rr is None:
                rr, ri = pr, pi
            else:
                rr, ri = rr * pr - ri * pi, rr * pi + ri * pr
        n >>= 1
        if n:
            pr, pi = pr * pr - pi * pi, 2.0 * pr * pi
    return rr, ri


def _cdiv(ar, ai, br, bi):
    swap = jnp.abs(br) < jnp.abs(bi)
    p = jnp.where(swap, bi, br)
    q = jnp.where(swap, br, bi)
    r = q / p
    den = p + q * r
    x = jnp.where(swap, ai, ar)
    y = jnp.where(swap, ar, ai)
    re = (x + y * r) / den
    im = (y - x * r) / den
    return re, jnp.where(swap, -im, im)


def _or_all(v):
    b = pltpu.bitcast(v, I32)
    n, d = b.shape
    parts = [b[r:r + 8, c:c + 128] for r in range(0, n, 8) for c in range(0, d, 128)]
    while len(parts) > 1:
        parts = [parts[i] | parts[i + 1] if i + 1 < len(parts) else parts[i]
                 for i in range(0, len(parts), 2)]
    return parts[0]


def _zero(b):
    return jnp.minimum(lax.shift_right_logical(b, 1), 0).astype(F32)


def _add_top(v, z):
    return jnp.concatenate([v[0:8, :] + z, v[8:, :]], axis=0)


def _kernel(x_hbm, lre_hbm, lim_hbm, ldt_hbm, dsk_hbm, bre_hbm, bim_hbm, cre_hbm, cim_hbm,
            w1t_hbm, w3t_hbm, w2_hbm, o_hbm,
            xv, lre_v, lim_v, ldt_v, dsk_v, wa, craw, cp, w2s,
            xs, xn_ref, base_cur, base_nxt, hh_ref, u_ref, g_ref, par_ref, dskf, carry_ref, ost0, ostl,
            sem, osem, *, L, D, P, F):
    NC = D // 128
    NLOOP = (L - T0) // T
    assert T0 + NLOOP * T == L
    FM = (F // 128) * 128
    FR = F - FM
    assert FM == 13 * 128 and 2 * FR == 128 and P == 5 * 128

    cnt = [0]

    def cp_(src, dst):
        c = pltpu.make_async_copy(src, dst, sem.at[cnt[0]])
        cnt[0] += 1
        return c

    rows = lambda ref, s, n: ref.at[pl.ds(s, n)]

    pos = [0]
    where = {}

    def wpiece(name, src, a, b):
        n = b - a
        c = cp_(rows(src, a, n), rows(wa, pos[0], n))
        where[name] = (pos[0], pos[0] + n)
        pos[0] += n
        return c

    c128 = lambda a: a * 128
    gv = [cp_(s, d) for s, d in [(dsk_hbm, dsk_v), (lre_hbm, lre_v), (lim_hbm, lim_v), (ldt_hbm, ldt_v)]]
    g0 = [cp_(rows(x_hbm, 0, T0), rows(xv, 0, T0))]
    g1 = [wpiece("g0", w1t_hbm, 0, c128(4))]
    e1 = pos[0]
    g2 = [wpiece("u0", w3t_hbm, 0, c128(4)), wpiece("g1", w1t_hbm, c128(4), c128(8))]
    e2 = pos[0]
    g3 = [wpiece("u1", w3t_hbm, c128(4), c128(8)), wpiece("g2", w1t_hbm, c128(8), c128(11)),
          wpiece("bre", bre_hbm, 0, P)]
    e3 = pos[0]
    g4 = [wpiece("bim", bim_hbm, 0, P), wpiece("u2", w3t_hbm, c128(8), c128(11)),
          wpiece("g3", w1t_hbm, c128(11), FM), wpiece("u3", w3t_hbm, c128(11), FM)]
    e4 = pos[0]
    g4 += [wpiece("gr", w1t_hbm, FM, F), wpiece("ur", w3t_hbm, FM, F)]
    e5 = pos[0]
    g5 = [cp_(w2_hbm, w2s), cp_(cre_hbm, craw.at[0]), cp_(cim_hbm, craw.at[1])]
    XS0 = cnt[0]
    B0 = where["bre"][0]
    B1 = where["bim"][1]

    def x_copy(k):
        s = T0 + k * T
        if not isinstance(k, int):
            s = pl.multiple_of(s, 16)
        return pltpu.make_async_copy(rows(x_hbm, s, T), rows(xv, s, T), sem.at[XS0 + k])

    def out_copy(k, c):
        if isinstance(k, int) and k < 0:
            src, start, n = ost0.at[c], 0, T0
        else:
            src, start, n = ostl.at[k, c], T0 + k * T, T
            if not isinstance(k, int):
                start = pl.multiple_of(start, 16)
        return pltpu.make_async_copy(
            src, o_hbm.at[pl.ds(start, n), pl.ds(c * 128, 128)], osem.at[k + 1])

    def ln_stage_in(start, n):
        xf = xv[pl.ds(start, n), :].astype(F32)
        for c in range(NC):
            xs[c, 0:n, :] = xf[:, c * 128:(c + 1) * 128]

    def ln_pieces(n, base_ref, q0, q1, ntok=0):
        seg = n // 8
        toks = [None] * ntok
        for q in range(q0, q1):
            j = 2 * q
            xp = jnp.concatenate(
                [jnp.concatenate([xs[c, pl.ds(jj, 8, stride=seg), :] for jj in (j, j + 1)], axis=0)
                 for c in range(NC)], axis=1)
            mean = jnp.mean(xp, axis=-1, keepdims=True)
            xc32 = xp - mean
            var = jnp.mean(xc32 * xc32, axis=-1, keepdims=True)
            den = _bf(jnp.sqrt(_bf(_bf(var) + 1e-5)))
            xnb = (_bf(xp - _bf(mean)) * (1.0 / den)).astype(BF16)
            xn_ref[j * 8:(j + 2) * 8, :] = xnb
            base = xp + xnb.astype(F32) * dskf[0:1, :]
            base_ref[j * 8:(j + 2) * 8, :] = base
            if ntok:
                p = (q - q0) * ntok // (q1 - q0)
                b = _or_all(base)
                toks[p] = b if toks[p] is None else toks[p] | b
        if ntok:
            toks = [_zero(t) for t in toks]
            return (jnp.concatenate(toks[0:NC], axis=1), jnp.concatenate(toks[NC:2 * NC], axis=1))

    def ln_next(start):
        ln_stage_in(start, T)
        return ln_pieces(T, base_nxt, 0, T // 16, 2 * NC)

    def param_stage():
        lre = lre_v[...].astype(F32).reshape(1, P)
        lim = lim_v[...].astype(F32).reshape(1, P)
        dt = _bf(jnp.exp(ldt_v[...].astype(F32).reshape(1, P)))
        er = jnp.exp(dt * lre)
        are = er * jnp.cos(dt * lim)
        aim = er * jnp.sin(dt * lim)
        kre, kim = _cdiv(are - 1.0, aim, lre, lim)
        par_ref[0] = jnp.broadcast_to(are, (8, P))
        par_ref[1] = jnp.broadcast_to(aim, (8, P))
        for t, off in ((T0, 2), (T, 8)):
            pr, pi = _cpow(are, aim, t // 8)
            for k in range(3):
                par_ref[off + 2 * k] = jnp.broadcast_to(pr, (8, P))
                par_ref[off + 1 + 2 * k] = jnp.broadcast_to(pi, (8, P))
                pr, pi = pr * pr - pi * pi, 2.0 * pr * pi
        par_ref[14] = jnp.broadcast_to(2.0 * kre, (8, P))
        par_ref[15] = jnp.broadcast_to(2.0 * kim, (8, P))
        carry_ref[...] = jnp.zeros_like(carry_ref)

    def cprep_stage():
        kre = par_ref[14, 0:1, :]
        kim = par_ref[15, 0:1, :]
        cre = craw[0].astype(F32)
        cim = craw[1].astype(F32)
        cp[:, 0:P] = (cre * kre - cim * kim).astype(BF16)
        cp[:, P:2 * P] = (-(cre * kim) - cim * kre).astype(BF16)

    def scan_stage(n, off):
        seg = n // 8
        are = par_ref[0]
        aim = par_ref[1]

        def park(slot, vr, vi):
            carry_ref[slot] = vr
            carry_ref[slot + 1] = vi
            return carry_ref[slot], carry_ref[slot + 1]

        er = u_ref[0:8, 0:P]
        ei = u_ref[0:8, P:2 * P]
        for j in range(1, seg):
            ur = u_ref[j * 8:(j + 1) * 8, 0:P]
            ui = u_ref[j * 8:(j + 1) * 8, P:2 * P]
            er, ei = (are * er - aim * ei) + ur, (are * ei + aim * er) + ui
            if j % PARK == 0:
                er, ei = park(2, er, ei)
        row = lax.broadcasted_iota(I32, (8, P), 0)
        zr = jnp.where(row == 0, pltpu.roll(carry_ref[0], 1, 0), pltpu.roll(er, 1, 0))
        zi = jnp.where(row == 0, pltpu.roll(carry_ref[1], 1, 0), pltpu.roll(ei, 1, 0))
        for k in range(3):
            d = 1 << k
            pr = par_ref[off + 2 * k]
            pi = par_ref[off + 1 + 2 * k]
            sr = jnp.where(row >= d, pltpu.roll(zr, d, 0), 0.0)
            si = jnp.where(row >= d, pltpu.roll(zi, d, 0), 0.0)
            zr, zi = zr + (pr * sr - pi * si), zi + (pr * si + pi * sr)
        hr, hi = zr, zi
        for j in range(0, seg, 2):
            if j % PARK == 0:
                hr, hi = park(0, hr, hi)
            outs_r = []
            outs_i = []
            for jj in (j, j + 1):
                ur = u_ref[jj * 8:(jj + 1) * 8, 0:P]
                ui = u_ref[jj * 8:(jj + 1) * 8, P:2 * P]
                hr, hi = (are * hr - aim * hi) + ur, (are * hi + aim * hr) + ui
                outs_r.append(hr)
                outs_i.append(hi)
            g_ref[j * 8:(j + 2) * 8, 0:P] = jnp.concatenate(outs_r, axis=0).astype(BF16)
            g_ref[j * 8:(j + 2) * 8, P:2 * P] = jnp.concatenate(outs_i, axis=0).astype(BF16)
        carry_ref[0] = hr
        carry_ref[1] = hi

    def out_stage(k, res):
        first = isinstance(k, int) and k < 0
        seg = (T0 if first else T) // 8
        for c in range(NC):
            for j in range(seg):
                v = res[j * 8:(j + 1) * 8, c * 128:(c + 1) * 128]
                if first:
                    ost0[c, pl.ds(j, 8, stride=seg), :] = v
                else:
                    ostl[k, c, pl.ds(j, 8, stride=seg), :] = v
            out_copy(k, c).start()

    def sl(r, base, name):
        a, b = where[name]
        return r[:, a - base:b - base]

    for grp in (gv, g0, g1, g2, g3, g4, g5):
        for c in grp:
            c.start()
    for k in range(NLOOP):
        x_copy(k).start()

    def wait(grp):
        for c in grp:
            c.wait()

    xdot = lambda a, b, r0=0, r1=T0: _dot_nt(xn_ref[r0:r1, :], wa[a:b, :])

    wait(gv)
    dskf[...] = jnp.broadcast_to(dsk_v[...].astype(F32).reshape(1, D), (8, D))
    param_stage()
    wait(g0)
    ln_stage_in(0, T0)
    NP0 = T0 // 16
    H = NP0 // 2
    ln_pieces(T0, base_cur, 0, H)
    wait(g1)
    ra = xdot(0, e1, 0, H * 16)
    ln_pieces(T0, base_cur, H, NP0)
    rb = xdot(0, e1, H * 16, T0)
    r1 = jnp.concatenate([ra, rb], axis=0)
    wait(g2)
    r2 = xdot(e1, e2)
    hh_ref[:, c128(0):c128(4)] = _silu_mul(r1, sl(r2, e1, "u0"))
    wait(g3)
    r3 = xdot(e2, e3)
    hh_ref[:, c128(4):c128(8)] = _silu_mul(sl(r2, e1, "g1"), sl(r3, e2, "u1"))
    u_ref[0:T0, 0:P] = sl(r3, e2, "bre")
    wait(g4)
    r4 = xdot(e3, e4)
    u_ref[0:T0, P:2 * P] = sl(r4, e3, "bim")
    scan_stage(T0, 2)
    qs = [0] + [((T0 * i // 4) + 15) // 16 * 16 for i in (1, 2, 3)] + [T0]
    rr = jnp.concatenate([xdot(e4, e5, qs[i], qs[i + 1]) for i in range(4)], axis=0)
    hh_ref[:, FM:F] = _silu_mul(rr[:, 0:FR], rr[:, FR:2 * FR])
    hh_ref[:, c128(8):c128(11)] = _silu_mul(sl(r3, e2, "g2"), sl(r4, e3, "u2"))
    hh_ref[:, c128(11):FM] = _silu_mul(sl(r4, e3, "g3"), sl(r4, e3, "u3"))
    wait(g5)
    x_copy(0).wait()
    cprep_stage()
    z1, z2 = ln_next(T0)
    acc = _add_top(base_cur[0:T0, :] + _dot(hh_ref[...], w2s[...]), z1)
    acc = _add_top(acc + _dot_nt(g_ref[0:T0, :], cp[...]), z2)
    out_stage(-1, acc)

    def body(k, carry):
        kn = jnp.minimum(k + 1, NLOOP - 1)

        @pl.when(k + 1 < NLOOP)
        def _():
            x_copy(kn).wait()

        nxt = pl.multiple_of(T0 + kn * T, 16)
        xnb = xn_ref[0:T, :]
        u_ref[0:T, :] = _dot_nt(xnb, wa[B0:B1, :])
        base_cur[0:T, :] = base_nxt[...]
        scan_stage(T, 8)
        ra = _dot_nt(xnb, wa[0:B0, :])
        rb = _dot_nt(xnb, wa[B1:e5, :])
        hh = jnp.concatenate([
            _silu_mul(sl(ra, 0, "g0"), sl(ra, 0, "u0")),
            _silu_mul(sl(ra, 0, "g1"), sl(ra, 0, "u1")),
            _silu_mul(sl(ra, 0, "g2"), sl(rb, B1, "u2")),
            _silu_mul(sl(rb, B1, "g3"), sl(rb, B1, "u3")),
            _silu_mul(sl(rb, B1, "gr"), sl(rb, B1, "ur")),
        ], axis=1)
        z1, z2 = ln_next(nxt)
        acc = _add_top(base_cur[0:T, :] + _dot(hh, w2s[...]), z1)
        acc = _add_top(acc + _dot_nt(g_ref[0:T, :], cp[...]), z2)
        out_stage(k, acc)
        return carry

    lax.fori_loop(0, NLOOP, body, 0)

    for k in range(-1, NLOOP):
        for c in range(NC):
            out_copy(k, c).wait()


@jax.jit
def pallas_parallel_sum__ssm_conv_s5__glu_gated_swiglu__prompt_kernel(
    A_x, A_Lambda_re, A_Lambda_im, A_B_re, A_B_im, A_C_re, A_C_im, A_log_dt, A_Dskip,
    B_x, B_w1, B_w3, B_w2,
):
    Bsz, L, D = A_x.shape
    P = A_Lambda_re.shape[0]
    F = B_w1.shape[1]
    NLOOP = (L - T0) // T
    TM = max(T0, T)
    hbm = pl.BlockSpec(memory_space=pltpu.HBM)
    out = pl.pallas_call(
        functools.partial(_kernel, L=L, D=D, P=P, F=F),
        in_specs=[hbm] * 12,
        out_specs=hbm,
        out_shape=jax.ShapeDtypeStruct((L, D), F32),
        scratch_shapes=[
            pltpu.VMEM((L, D), BF16),
            pltpu.VMEM((P,), BF16), pltpu.VMEM((P,), BF16), pltpu.VMEM((P,), BF16), pltpu.VMEM((D,), BF16),
            pltpu.VMEM((2 * P + 2 * F, D), BF16),
            pltpu.VMEM((2, D, P), BF16),
            pltpu.VMEM((D, 2 * P), BF16),
            pltpu.VMEM((F, D), BF16),
            pltpu.VMEM((D // 128, TM, 128), F32),
            pltpu.VMEM((TM, D), BF16),
            pltpu.VMEM((TM, D), F32),
            pltpu.VMEM((T, D), F32),
            pltpu.VMEM((T0, F), BF16),
            pltpu.VMEM((TM, 2 * P), F32),
            pltpu.VMEM((TM, 2 * P), BF16),
            pltpu.VMEM((16, 8, P), F32),
            pltpu.VMEM((8, D), F32),
            pltpu.VMEM((4, 8, P), F32),
            pltpu.VMEM((D // 128, T0, 128), F32),
            pltpu.VMEM((NLOOP, D // 128, T, 128), F32),
            pltpu.SemaphoreType.DMA((20 + NLOOP,)),
            pltpu.SemaphoreType.DMA((NLOOP + 1,)),
        ],
        compiler_params=pltpu.CompilerParams(
            vmem_limit_bytes=100 * 1024 * 1024,
            disable_bounds_checks=True,
            disable_semaphore_checks=True,
        ),
    )(A_x.reshape(L, D), A_Lambda_re, A_Lambda_im, A_log_dt, A_Dskip,
      A_B_re, A_B_im, A_C_re, A_C_im, B_w1.T, B_w3.T, B_w2)
    return out.reshape(Bsz, L, D)
```
